```python
import jax
import jax.numpy as jnp

def _softmax(x, axis=-1):
    return jax.nn.softmax(x, axis=axis)
def _gelu(x):
    return jax.nn.gelu(x, approximate=True)
def _silu(x):
    return jax.nn.silu(x)
def _sigmoid(x):
    return jax.nn.sigmoid(x)
def _layernorm(x, axis=-1, eps=1e-5):
    m = jnp.mean(x, axis=axis, keepdims=True)
    v = jnp.var(x, axis=axis, keepdims=True)
    return (x - m) / jnp.sqrt(v + eps)
def _scatter_add(tgt, idx, src, axis=0):
    return tgt.at[idx].add(src)
def _segment_sum(src, seg, n):
    return jax.ops.segment_sum(src, seg, n)
class _Rng:
    def __init__(self, key):
        self._k = key
    def _next(self):
        self._k, sub = jax.random.split(self._k)
        return sub
    def normal(self, shape):
        return jax.random.normal(self._next(), shape, dtype=jnp.bfloat16)
    def randint(self, lo, hi, shape):
        return jax.random.randint(self._next(), shape, lo, hi, dtype=jnp.int32)
    def uniform(self, shape, lo=0.0, hi=1.0):
        return jax.random.uniform(self._next(), shape, jnp.bfloat16, lo, hi)
    def permutation(self, n):
        return jax.random.permutation(self._next(), n)


kernel_name = 'gated_mix__sliding_block_cached__moe_arch_mod__decode'

def setup_inputs():
    _rng = _Rng(jax.random.key(int.from_bytes(__import__("os").urandom(4), "little")))
    _w = (lambda a: (lambda t: t.astype(jnp.bfloat16) if jnp.issubdtype(t.dtype, jnp.floating) else t)(jnp.asarray(a)))
    def _A_setup():
        B, Sq, D = 1, 1, 640
        Hq, Hkv, Sk, Dh = 32, 32, 32768, 192
        assert Hq % Hkv == 0, (Hq, Hkv)
        return {
            "x": _w((lambda *s: _rng.normal(s) * 0.05)(B, Sq, D)),
            "k_cache": _w((lambda *s: _rng.normal(s) * 0.05)(B, Hkv, Sk, Dh)),
            "v_cache": _w((lambda *s: _rng.normal(s) * 0.05)(B, Hkv, Sk, Dh)),
            "wq": _w((lambda *s: _rng.normal(s) * 0.05)(D, Hq * Dh) * (D ** -0.5)),
            "wo": _w((lambda *s: _rng.normal(s) * 0.05)(Hq * Dh, D) * ((Hq * Dh) ** -0.5)),
        }
    _A_in = _A_setup()

    def _B_setup():
        B, S, D, F, C = 1, 1, 640, 1536, 1
        return {
            "x": _w((lambda *s: _rng.normal(s) * 0.05)(B, S, D)),
            "w_r": _w((lambda *s: _rng.normal(s) * 0.05)(D)),
            "w_gate": _w((lambda *s: _rng.normal(s) * 0.05)(D, F)),
            "w_up": _w((lambda *s: _rng.normal(s) * 0.05)(D, F)),
            "w_down": _w((lambda *s: _rng.normal(s) * 0.05)(F, D)),
        }
    _B_in = _B_setup()

    return {
        "A_x": _A_in["x"],
        "A_k_cache": _A_in["k_cache"],
        "A_v_cache": _A_in["v_cache"],
        "A_wq": _A_in["wq"],
        "A_wo": _A_in["wo"],
        "B_x": _B_in["x"],
        "B_w_r": _B_in["w_r"],
        "B_w_gate": _B_in["w_gate"],
        "B_w_up": _B_in["w_up"],
        "B_w_down": _B_in["w_down"],
        "gate_w": _w((lambda *s: _rng.normal(s) * 0.05)(640)),
    }

def reference(A_x, A_k_cache, A_v_cache, A_wq, A_wo, B_x, B_w_r, B_w_gate, B_w_up, B_w_down, gate_w):
    def _A_ref(x, k_cache, v_cache, wq, wo):
        B, Sq, D = x.shape
        Hq, Dh = 32, 192
        Hkv, Sk = k_cache.shape[1], k_cache.shape[2]
        W = min(4096, max(256, Sk // 4))
        rep = Hq // Hkv
        q = (lambda x, *d: x.transpose(*d))((x @ wq).reshape(B, Sq, Hq, Dh), 0, 2, 1, 3)
        k = jnp.repeat(k_cache[:, :, Sk - W:, :], rep, axis=1)
        v = jnp.repeat(v_cache[:, :, Sk - W:, :], rep, axis=1)
        scores = jnp.einsum("bhqd,bhkd->bhqk", q, k) * (Dh ** -0.5)
        p = _softmax(scores, axis=-1)
        o = jnp.einsum("bhqk,bhkd->bhqd", p, v)
        return (lambda x, *d: x.transpose(*d))(o, 0, 2, 1, 3).reshape(B, Sq, Hq * Dh) @ wo

    def _B_ref(x, w_r, w_gate, w_up, w_down):
        B, S, D = x.shape
        C = 1
        r = x @ w_r
        idx = jnp.argsort(-r, axis=-1)[:, :C]
        idx_e = jnp.repeat(idx.reshape(B, C, 1), D, axis=2)
        x_sel = jnp.take_along_axis(x, idx_e, axis=1)
        g = _silu(x_sel @ w_gate)
        u = x_sel @ w_up
        y = (g * u) @ w_down
        r_sel = _sigmoid(jnp.take_along_axis(r, idx, axis=1))
        y = y * r_sel.reshape(B, C, 1)
        b_off = (jnp.arange(B) * S).reshape(B, 1)
        flat_idx = (idx + b_off).reshape(B * C)
        zero = (x * 0.0).reshape(B * S, D)
        upd = _scatter_add(zero, flat_idx, y.reshape(B * C, D), axis=0)
        return x + upd.reshape(B, S, D)

    x = A_x
    g = _sigmoid((x * gate_w).sum(-1, keepdims=True))
    a = _A_ref(x, A_k_cache, A_v_cache, A_wq, A_wo)
    b = _B_ref(x, B_w_r, B_w_gate, B_w_up, B_w_down)
    return g * a + (1 - g) * b
```

```python
import functools
import jax
import jax.numpy as jnp
import numpy as np
from jax import lax
from jax.experimental import pallas as pl
from jax.experimental.pallas import tpu as pltpu

H, DH, SK, W, D, F = 32, 192, 32768, 4096, 640, 1536
PD = 2 * DH
NP = H // 2
CR = 128
NCK = PD // CR
M = 8
BF = jnp.bfloat16
F32 = jnp.float32
NT = (((1,), (1,)), ((), ()))


def make(name="gmix", cap=192, kv_piece=(8, 2048), kv_order='cr', wo_rows=32, wo_blk=128, ffn_first=True,
         cp=None, scopes=False, interleave=False, wg_rows=8, wq_order='rc'):
  NS = 2 * NCK

  def scope(n):
    return jax.named_scope(n) if scopes else _null()

  def pieces(nr, nc, pr, pc, order):
    if order == 'rc':
      return [(a * pr, b * pc) for a in range(nr // pr) for b in range(nc // pc)]
    return [(a * pr, b * pc) for b in range(nc // pc) for a in range(nr // pr)]

  def kernel(x_hbm, kt, vt, wq, wo, wr_hbm, wg, wu, wd, gw_hbm, out_ref,
             x_v, wr_v, gw_v, ring, wq_v, wo_v, wg_v, wu_v, wd_v, q_v, o_v,
             ring_sem, small_sem, wq_sem, wo_sem, ffn_sem, wd_sem):

    class Block:
      def __init__(self, starts, wait):
        self.starts = starts
        self.wait = wait
        self.n = len(starts)

    def issue(blk):
      for k, s in enumerate(blk.starts):
        s(k % 2)

    def cp_piece(src, dst, sem, sr, sc, dr, dc, nr, nc):
      def go(p):
        pltpu.make_async_copy(src.at[pl.ds(sr, nr), pl.ds(sc, nc)],
                              dst.at[pl.ds(dr, nr), pl.ds(dc, nc)], sem).start(priority=p)
      return go

    def kv_block(src, j, i, slot):
      pr, pc = kv_piece
      r0 = j * PD + i * CR
      st = []
      for a, b in pieces(CR, W, pr, pc, kv_order):
        sr = r0 + a
        if not isinstance(sr, int):
          sr = pl.multiple_of(sr, 8)
        st.append(cp_piece(src, ring.at[slot], ring_sem.at[slot], sr, SK - W + b, a, b, pr, pc))
      return Block(st, lambda: pltpu.make_async_copy(ring.at[slot], ring.at[slot], ring_sem.at[slot]).wait())

    def row_block(pairs, sem, r0, nr, pr, pc, order='rc'):
      st = []
      for src, dst in pairs:
        for a, b in pieces(nr, src.shape[1], pr, pc, order):
          st.append(cp_piece(src, dst, sem, r0 + a, b, r0 + a, b, pr, pc))
      def wait():
        for src, dst in pairs:
          v = dst.at[pl.ds(r0, nr)]
          pltpu.make_async_copy(v, v, sem).wait()
      return Block(st, wait)

    small = [pltpu.make_async_copy(s, d, small_sem.at[i]) for i, (s, d) in
             enumerate([(x_hbm, x_v), (wr_hbm, wr_v), (gw_hbm, gw_v)])]
    gu_blocks = [row_block([(wg, wg_v), (wu, wu_v)], ffn_sem.at[i], CR * i, CR, wg_rows, F) for i in range(D // CR)]
    WDB = 384
    wd_blocks = [row_block([(wd, wd_v)], wd_sem.at[i], WDB * i, WDB, wo_rows, D) for i in range(F // WDB)]
    wq_blocks = [row_block([(wq, wq_v)], wq_sem.at[i], CR * i, CR, 8, 2048, wq_order) for i in range(D // CR)]
    fill = [kv_block(kt, 0, i, i) for i in range(NCK)] + [kv_block(vt, 0, i, NCK + i) for i in range(NCK)]
    wo_blocks = [row_block([(wo, wo_v)], wo_sem.at[i], wo_blk * i, wo_blk, wo_rows, D) for i in range(H * DH // wo_blk)]

    if ffn_first:
      stream = gu_blocks + wd_blocks + wq_blocks + fill
    else:
      stream = wq_blocks + gu_blocks + wd_blocks + fill
    state = dict(next=0, inflight=0)

    def pump():
      while state['next'] < len(stream) and state['inflight'] + stream[state['next']].n <= cap:
        b = stream[state['next']]
        issue(b)
        state['inflight'] += b.n
        state['next'] += 1

    def consume(b):
      b.wait()
      state['inflight'] -= b.n
      pump()

    for c in small:
      c.start()
    pump()
    for c in small:
      c.wait()
    x1 = x_v[...]
    x8 = jnp.broadcast_to(x1.astype(F32), (M, D)).astype(BF)

    res = {}

    def do_ffn():
      hg = None
      hu = None
      for i in range(D // CR):
        consume(gu_blocks[i])
        xs = x8[:, CR * i:CR * (i + 1)]
        dg = jnp.dot(xs, wg_v[pl.ds(CR * i, CR), :], preferred_element_type=F32)
        du = jnp.dot(xs, wu_v[pl.ds(CR * i, CR), :], preferred_element_type=F32)
        hg = dg if hg is None else hg + dg
        hu = du if hu is None else hu + du
      hg = hg.astype(BF).astype(F32)
      hu = hu.astype(BF).astype(F32)
      sg = jax.nn.sigmoid(hg).astype(BF).astype(F32)
      act = (hg * sg).astype(BF).astype(F32)
      gu = (act * hu).astype(BF)
      y = None
      for i in range(F // WDB):
        consume(wd_blocks[i])
        d = jnp.dot(gu[:, WDB * i:WDB * (i + 1)], wd_v[pl.ds(WDB * i, WDB), :], preferred_element_type=F32)
        y = d if y is None else y + d
      res['y'] = y.astype(BF).astype(F32)

    def do_q():
      q = None
      for i in range(D // CR):
        consume(wq_blocks[i])
        d = jnp.dot(x8[:, CR * i:CR * (i + 1)], wq_v[pl.ds(CR * i, CR), :], preferred_element_type=F32)
        q = d if q is None else q + d
      q_v[...] = q

    with scope("prologue"):
      if ffn_first:
        do_ffn()
        do_q()
      else:
        do_q()
        do_ffn()
    assert state['next'] == len(stream), state

    row = lax.broadcasted_iota(jnp.int32, (M, PD), 0)
    col = lax.broadcasted_iota(jnp.int32, (M, PD), 1)
    own = (row < M // 2) == (col < DH)
    scale = float(np.float32(DH ** -0.5).astype(BF).astype(np.float32))

    wo_starts = [s for b in wo_blocks for s in b.starts]
    per = -(-len(wo_starts) // NS)

    def refill(j, src, i, slot):
      @pl.when(j + 1 < NP)
      def _():
        issue(kv_block(src, j + 1, i, slot))

      @pl.when(j + 1 == NP)
      def _():
        for k, s in enumerate(wo_starts[slot * per:(slot + 1) * per]):
          s(k % 2)

    def pair(j, carry):
      c0 = pl.multiple_of(j * PD, CR)
      qm = jnp.where(own, q_v[:, pl.ds(c0, PD)], 0.0).astype(BF)
      s = None
      for i in range(NCK):
        slot = i
        pltpu.make_async_copy(ring.at[slot], ring.at[slot], ring_sem.at[slot]).wait()
        d = jnp.dot(qm[:, CR * i:CR * (i + 1)], ring[slot], preferred_element_type=F32)
        s = d if s is None else s + d
        refill(j, kt, i, slot)
      s = s.astype(BF).astype(F32) * scale
      s = s.astype(BF).astype(F32)
      m = jnp.max(s, axis=1, keepdims=True)
      e = jnp.exp(s - m)
      eb = e.astype(BF)
      l = jnp.sum(eb.astype(F32), axis=1, keepdims=True)
      inv = 1.0 / l
      os_ = []
      for i in range(NCK):
        slot = NCK + i
        pltpu.make_async_copy(ring.at[slot], ring.at[slot], ring_sem.at[slot]).wait()
        os_.append(lax.dot_general(eb, ring[slot], NT, preferred_element_type=F32))
        refill(j, vt, i, slot)
      o = jnp.concatenate(os_, axis=1) * inv
      o_v[:, pl.ds(c0, PD)] = jnp.where(own, o, 0.0)
      return carry

    with scope("main"):
      lax.fori_loop(0, NP, pair, 0)

    y = res['y']
    xf = x1.astype(F32)
    wr = wr_v[...].astype(F32)
    gw = gw_v[...].astype(F32)
    racc = jnp.zeros((1, 128), F32)
    gacc = jnp.zeros((1, 128), F32)
    for i in range(D // 128):
      xi = xf[:, 128 * i:128 * (i + 1)]
      racc = racc + xi * wr[i:i + 1, :]
      gacc = gacc + (xi * gw[i:i + 1, :]).astype(BF).astype(F32)
    r = jnp.sum(racc, axis=1, keepdims=True).astype(BF).astype(F32)
    gl = jnp.sum(gacc, axis=1, keepdims=True).astype(BF).astype(F32)
    r_sel = jax.nn.sigmoid(r).astype(BF).astype(F32)
    g = jax.nn.sigmoid(gl).astype(BF).astype(F32)
    y0 = (y[0:1] * r_sel).astype(BF).astype(F32)
    upd = (xf * 0.0 + y0).astype(BF).astype(F32)
    bb = (xf + upd).astype(BF).astype(F32)
    omg = (1.0 - g).astype(BF).astype(F32)
    t2 = (omg * bb).astype(BF).astype(F32)

    with scope("wo"):
      acc = None
      for j, b in enumerate(wo_blocks):
        b.wait()
        d = jnp.dot(o_v[:, wo_blk * j:wo_blk * (j + 1)].astype(BF), wo_v[pl.ds(wo_blk * j, wo_blk), :],
                    preferred_element_type=F32)
        acc = d if acc is None else acc + d
      a = (acc[0:1] + acc[M // 2:M // 2 + 1]).astype(BF).astype(F32)
      t1 = (g * a).astype(BF).astype(F32)
      out_ref[...] = (t1 + t2).astype(BF)

  def fn(A_x, kc, vc, wq, wo, B_x, w_r, wg, wu, wd, gw):
    kt = jnp.swapaxes(kc[0], 1, 2).reshape(H * DH, SK)
    vt = jnp.swapaxes(vc[0], 1, 2).reshape(H * DH, SK)
    hbm = pl.BlockSpec(memory_space=pltpu.HBM)
    out = pl.pallas_call(
        kernel,
        out_shape=jax.ShapeDtypeStruct((1, D), BF),
        in_specs=[hbm] * 10,
        out_specs=pl.BlockSpec(memory_space=pltpu.VMEM),
        scratch_shapes=[
            pltpu.VMEM((1, D), BF), pltpu.VMEM((5, 128), BF), pltpu.VMEM((5, 128), BF),
            pltpu.VMEM((NS, CR, W), BF),
            pltpu.VMEM((D, H * DH), BF), pltpu.VMEM((H * DH, D), BF),
            pltpu.VMEM((D, F), BF), pltpu.VMEM((D, F), BF), pltpu.VMEM((F, D), BF),
            pltpu.VMEM((M, H * DH), F32), pltpu.VMEM((M, H * DH), F32),
            pltpu.SemaphoreType.DMA((NS,)), pltpu.SemaphoreType.DMA((3,)),
            pltpu.SemaphoreType.DMA((D // CR,)), pltpu.SemaphoreType.DMA((H * DH // wo_blk,)),
            pltpu.SemaphoreType.DMA((D // CR,)), pltpu.SemaphoreType.DMA((F // 384,)),
        ],
        compiler_params=pltpu.CompilerParams(vmem_limit_bytes=100 * 1024 * 1024, **(cp or {})),
        name=name,
    )(A_x.reshape(1, D), kt, vt, wq, wo, w_r.reshape(5, 128), wg, wu, wd, gw.reshape(5, 128))
    return out.reshape(1, 1, D)

  return fn


class _null:
  def __enter__(self):
    return self

  def __exit__(self, *a):
    return False


_IMPL = make(name="gated_mix_decode", wo_rows=24, wo_blk=384)


@jax.jit
def pallas_gated_mix__sliding_block_cached__moe_arch_mod__decode_kernel(
    A_x: jax.Array,
    A_k_cache: jax.Array,
    A_v_cache: jax.Array,
    A_wq: jax.Array,
    A_wo: jax.Array,
    B_x: jax.Array,
    B_w_r: jax.Array,
    B_w_gate: jax.Array,
    B_w_up: jax.Array,
    B_w_down: jax.Array,
    gate_w: jax.Array,
):
  return _IMPL(A_x, A_k_cache, A_v_cache, A_wq, A_wo, B_x, B_w_r, B_w_gate, B_w_up, B_w_down, gate_w)
```

```python
import math
import jax
import jax.numpy as jnp
import numpy as np
from jax import lax
from jax.experimental import pallas as pl
from jax.experimental.pallas import tpu as pltpu

H, DH, SK, W, D, F = 32, 192, 32768, 4096, 640, 1536
PD = 2 * DH
NP = H // 2
CR = 128
NCK = PD // CR
NS = 2 * NCK
M = 8
BF = jnp.bfloat16
F32 = jnp.float32
NT = (((1,), (1,)), ((), ()))
SCALE = float(np.asarray(DH ** -0.5, np.float32).astype(BF).astype(np.float32))


def perm_of(P, S):
  if S == 1:
    return list(range(P))
  if math.gcd(S, P) == 1:
    return [(k * S) % P for k in range(P)]
  assert P % S == 0
  return [(k % (P // S)) * S + k // (P // S) for k in range(P)]


def rnd(x):
  return x.astype(BF).astype(F32)


def make(name="gmix", cap=256, kv_order='cr', gu_S=20, wd_rows=24, wd_S=8, wq_S=12, wq_ng=2,
         wo_rows=24, wo_groups=((128, 16), (64, 8), (32, 8), (32, 8)), order='fq',
         cp=None, scopes=False, semchk=False, flip=0):

  def scope(n):
    return jax.named_scope(n) if scopes else _null()

  def kv_pieces():
    nr, nc = CR // 8, 2
    if kv_order == 'rc':
      l = [(a, b) for a in range(nr) for b in range(nc)]
    elif kv_order == 'cr':
      l = [(a, b) for b in range(nc) for a in range(nr)]
    elif kv_order == 'diag':
      l = [(a, (a + b) % nc) for b in range(nc) for a in range(nr)]
    elif kv_order == 's3':
      l = [((3 * a) % nr, b) for b in range(nc) for a in range(nr)]
    return [(8 * a, 2048 * b) for a, b in l]

  assert sum(g[0] for g in wo_groups) * wo_rows == H * DH

  def kernel(x_hbm, kt, vt, wq, wo, wr_hbm, wg, wu, wd, gw_hbm, out_ref,
             x_v, wr_v, gw_v, ring, wq_v, wo_v, wg_v, wu_v, wd_v, q_v, o_v,
             ring_sem, small_sem, wq_sem, wo_sem, ffn_sem):

    class Group:
      def __init__(self, descs, waits):
        self.descs = descs
        self.waits = waits
        self.n = len(descs)

      def issue(self):
        for k, d in enumerate(self.descs):
          d().start(priority=(k + flip) % 2)

      def wait(self):
        for v, s in self.waits:
          pltpu.make_async_copy(v, v, s).wait()

    def piece(src, dst, sem, sr, sc, dr, dc, nr, nc):
      return lambda: pltpu.make_async_copy(src.at[pl.ds(sr, nr), pl.ds(sc, nc)],
                                           dst.at[pl.ds(dr, nr), pl.ds(dc, nc)], sem)

    def kv_block(src, j, i, slot):
      r0 = j * PD + i * CR
      st = []
      for a, b in kv_pieces():
        sr = r0 + a
        if not isinstance(sr, int):
          sr = pl.multiple_of(sr, 8)
        st.append(piece(src, ring.at[slot], ring_sem.at[slot], sr, SK - W + b, a, b, 8, 2048))
      return Group(st, [(ring.at[slot], ring_sem.at[slot])])

    def rows_group(src, dst, sem, r0, n, pr, pc, S):
      per_row = src.shape[1] // pc
      ds_ = []
      for u in perm_of(n, S):
        a, b = r0 + pr * (u // per_row), pc * (u % per_row)
        ds_.append(piece(src, dst, sem, a, b, a, b, pr, pc))
      return Group(ds_, [(dst.at[pl.ds(r0, pr * (n // per_row))], sem)])

    small = [pltpu.make_async_copy(s, d, small_sem.at[i]) for i, (s, d) in
             enumerate([(x_hbm, x_v), (wr_hbm, wr_v), (gw_hbm, gw_v)])]
    g_g = rows_group(wg, wg_v, ffn_sem.at[0], 0, 80, 8, F, gu_S)
    g_u = rows_group(wu, wu_v, ffn_sem.at[1], 0, 80, 8, F, gu_S)
    gu = Group([d for pr in zip(g_g.descs, g_u.descs) for d in pr], g_g.waits + g_u.waits)
    g_d = rows_group(wd, wd_v, ffn_sem.at[2], 0, F // wd_rows, wd_rows, D, wd_S)
    wq_groups = [rows_group(wq, wq_v, wq_sem.at[g], g * (D // wq_ng), 240 // wq_ng, 8, 2048, wq_S) for g in range(wq_ng)]
    fill = [kv_block(kt, 0, i, i) for i in range(NCK)] + [kv_block(vt, 0, i, NCK + i) for i in range(NCK)]
    wo_grps = []
    t0 = 0
    for gi, (n, S) in enumerate(wo_groups):
      wo_grps.append((rows_group(wo, wo_v, wo_sem.at[gi], wo_rows * t0, n, wo_rows, D, S), wo_rows * t0, wo_rows * n))
      t0 += n

    if order == 'fq':
      stream = [gu, g_d] + wq_groups + fill
    else:
      stream = wq_groups + [gu, g_d] + fill
    state = dict(next=0, inflight=0)

    def pump(once=False):
      while state['next'] < len(stream) and state['inflight'] + stream[state['next']].n <= cap:
        b = stream[state['next']]
        b.issue()
        state['inflight'] += b.n
        state['next'] += 1
        if once:
          break

    def consume(b):
      b.wait()
      state['inflight'] -= b.n
      pump()

    with scope("s_pump"):
      pump(once=True)
      for c in small:
        c.start()
      pump()
      for c in small:
        c.wait()
    x1 = x_v[...]
    x8 = jnp.broadcast_to(x1.astype(F32), (M, D)).astype(BF)

    res = {}

    def do_ffn():
      with scope("gu"):
        consume(gu)
      hg = rnd(jnp.dot(x8, wg_v[...], preferred_element_type=F32))
      hu = rnd(jnp.dot(x8, wu_v[...], preferred_element_type=F32))
      act = rnd(hg * rnd(jax.nn.sigmoid(hg)))
      gub = (act * hu).astype(BF)
      with scope("wd"):
        consume(g_d)
      res['y'] = rnd(jnp.dot(gub, wd_v[...], preferred_element_type=F32))

    def do_q():
      q = None
      nr = D // wq_ng
      for i, g in enumerate(wq_groups):
        with scope(f"wq{i}"):
          consume(g)
        if wq_ng in (1, 5):
          d = jnp.dot(x8[:, nr * i:nr * (i + 1)], wq_v[pl.ds(nr * i, nr), :], preferred_element_type=F32)
          q = d if q is None else q + d
      if q is None:
        q = jnp.dot(x8, wq_v[...], preferred_element_type=F32)
      q_v[...] = q

    with scope("prologue"):
      if order == 'fq':
        do_ffn()
        do_q()
      else:
        do_q()
        do_ffn()
    assert state['next'] == len(stream), state

    row = lax.broadcasted_iota(jnp.int32, (M, PD), 0)
    col = lax.broadcasted_iota(jnp.int32, (M, PD), 1)
    own = (row < M // 2) == (col < DH)

    wo_descs = [d for (g, _, _) in wo_grps for d in g.descs]
    per = -(-len(wo_descs) // NS)

    def refill(j, src, i, slot):
      @pl.when(j + 1 < NP)
      def _():
        kv_block(src, j + 1, i, slot).issue()

      @pl.when(j + 1 == NP)
      def _():
        for k, d in list(enumerate(wo_descs))[slot * per:(slot + 1) * per]:
          d().start(priority=(k + flip) % 2)

    def pair(j, carry):
      c0 = pl.multiple_of(j * PD, CR)
      qm = jnp.where(own, q_v[:, pl.ds(c0, PD)], 0.0).astype(BF)
      s = None
      for i in range(NCK):
        slot = i
        pltpu.make_async_copy(ring.at[slot], ring.at[slot], ring_sem.at[slot]).wait()
        d = jnp.dot(qm[:, CR * i:CR * (i + 1)], ring[slot], preferred_element_type=F32)
        s = d if s is None else s + d
        refill(j, kt, i, slot)
      s = rnd(rnd(s) * SCALE)
      m = jnp.max(s, axis=1, keepdims=True)
      eb = jnp.exp(s - m).astype(BF)
      l = jnp.sum(eb.astype(F32), axis=1, keepdims=True)
      inv = 1.0 / l
      os_ = []
      for i in range(NCK):
        slot = NCK + i
        pltpu.make_async_copy(ring.at[slot], ring.at[slot], ring_sem.at[slot]).wait()
        os_.append(lax.dot_general(eb, ring[slot], NT, preferred_element_type=F32))
        refill(j, vt, i, slot)
      o = jnp.concatenate(os_, axis=1) * inv
      o_v[:, pl.ds(c0, PD)] = jnp.where(own, o, 0.0)
      return carry

    with scope("main"):
      lax.fori_loop(0, NP, pair, 0)

    y = res['y']
    xf = x1.astype(F32)
    wr = wr_v[...].astype(F32)
    gw = gw_v[...].astype(F32)
    racc = jnp.zeros((1, 128), F32)
    gacc = jnp.zeros((1, 128), F32)
    for i in range(D // 128):
      xi = xf[:, 128 * i:128 * (i + 1)]
      racc = racc + xi * wr[i:i + 1, :]
      gacc = gacc + rnd(xi * gw[i:i + 1, :])
    r = rnd(jnp.sum(racc, axis=1, keepdims=True))
    gl = rnd(jnp.sum(gacc, axis=1, keepdims=True))
    r_sel = rnd(jax.nn.sigmoid(r))
    g = rnd(jax.nn.sigmoid(gl))
    y0 = rnd(y[0:1] * r_sel)
    upd = rnd(xf * 0.0 + y0)
    bb = rnd(xf + upd)
    t2 = rnd(rnd(1.0 - g) * bb)

    with scope("wo"):
      acc = None
      for gi, (grp, r0, nr) in enumerate(wo_grps):
        with scope(f"wo{gi}"):
          grp.wait()
        d = jnp.dot(o_v[:, r0:r0 + nr].astype(BF), wo_v[pl.ds(r0, nr), :], preferred_element_type=F32)
        acc = d if acc is None else acc + d
      a = rnd(acc[0:1] + acc[M // 2:M // 2 + 1])
      out_ref[...] = (rnd(g * a) + t2).astype(BF)

  def fn(A_x, kc, vc, wq, wo, B_x, w_r, wg, wu, wd, gw):
    kt = jnp.swapaxes(kc[0], 1, 2).reshape(H * DH, SK)
    vt = jnp.swapaxes(vc[0], 1, 2).reshape(H * DH, SK)
    hbm = pl.BlockSpec(memory_space=pltpu.HBM)
    out = pl.pallas_call(
        kernel,
        out_shape=jax.ShapeDtypeStruct((1, D), BF),
        in_specs=[hbm] * 10,
        out_specs=pl.BlockSpec(memory_space=pltpu.VMEM),
        scratch_shapes=[
            pltpu.VMEM((1, D), BF), pltpu.VMEM((5, 128), BF), pltpu.VMEM((5, 128), BF),
            pltpu.VMEM((NS, CR, W), BF),
            pltpu.VMEM((D, H * DH), BF), pltpu.VMEM((H * DH, D), BF),
            pltpu.VMEM((D, F), BF), pltpu.VMEM((D, F), BF), pltpu.VMEM((F, D), BF),
            pltpu.VMEM((M, H * DH), F32), pltpu.VMEM((M, H * DH), F32),
            pltpu.SemaphoreType.DMA((NS,)), pltpu.SemaphoreType.DMA((3,)),
            pltpu.SemaphoreType.DMA((wq_ng,)), pltpu.SemaphoreType.DMA((len(wo_groups),)),
            pltpu.SemaphoreType.DMA((3,)),
        ],
        compiler_params=pltpu.CompilerParams(vmem_limit_bytes=64 * 1024 * 1024,
                                             disable_semaphore_checks=not semchk, **(cp or {})),
        name=name,
    )(A_x.reshape(1, D), kt, vt, wq, wo, w_r.reshape(5, 128), wg, wu, wd, gw.reshape(5, 128))
    return out.reshape(1, 1, D)

  return fn


class _null:
  def __enter__(self):
    return self

  def __exit__(self, *a):
    return False


_IMPL = make(name="gated_mix_decode")


@jax.jit
def pallas_gated_mix__sliding_block_cached__moe_arch_mod__decode_kernel(
    A_x: jax.Array,
    A_k_cache: jax.Array,
    A_v_cache: jax.Array,
    A_wq: jax.Array,
    A_wo: jax.Array,
    B_x: jax.Array,
    B_w_r: jax.Array,
    B_w_gate: jax.Array,
    B_w_up: jax.Array,
    B_w_down: jax.Array,
    gate_w: jax.Array,
):
  return _IMPL(A_x, A_k_cache, A_v_cache, A_wq, A_wo, B_x, B_w_r, B_w_gate, B_w_up, B_w_down, gate_w)
```

```python
import math

import jax
import jax.numpy as jnp
import numpy as np
from jax import lax
import jax.experimental.pallas as pl
import jax.experimental.pallas.tpu as pltpu

H, DH, SK, W, D, F = 32, 192, 32768, 4096, 640, 1536
PD = 2 * DH
NP = H // 2
HW = W // 2
NS = 4
M = 8
CAP = 256
BF = jnp.bfloat16
F32 = jnp.float32
NT = (((1,), (1,)), ((), ()))
SCALE = float(np.asarray(DH ** -0.5, np.float32).astype(BF).astype(np.float32))

GU_S, WD_S, WQ_S = 20, 8, 12
WQ_NG = 2
WR = 24
WO_GROUPS = ((128, 16), (64, 8), (32, 8), (16, 8), (16, 8))


def _perm(n, stride):
  if math.gcd(stride, n) == 1:
    return [(k * stride) % n for k in range(n)]
  return [(k % (n // stride)) * stride + k // (n // stride) for k in range(n)]


def _rnd(x):
  return x.astype(BF).astype(F32)


def _piece(src, dst, sem, sr, sc, dr, dc, nr, nc):
  return lambda: pltpu.make_async_copy(
      src.at[pl.ds(sr, nr), pl.ds(sc, nc)], dst.at[pl.ds(dr, nr), pl.ds(dc, nc)], sem)


def _start_all(descs, k0=0):
  for k, d in enumerate(descs):
    d().start(priority=(k0 + k + 1) % 2)


def _wait_all(ref, sem):
  pltpu.make_async_copy(ref, ref, sem).wait()


class _Group:
  def __init__(self, descs, waits):
    self.descs = descs
    self.waits = waits
    self.n = len(descs)

  def issue(self):
    _start_all(self.descs)

  def wait(self):
    for ref, sem in self.waits:
      _wait_all(ref, sem)


def _rows_group(src, dst, sem, r0, n, pr, pc, stride):
  per_row = src.shape[1] // pc
  descs = []
  for u in _perm(n, stride):
    a, b = r0 + pr * (u // per_row), pc * (u % per_row)
    descs.append(_piece(src, dst, sem, a, b, a, b, pr, pc))
  return _Group(descs, [(dst.at[pl.ds(r0, pr * (n // per_row))], sem)])


def _kernel(x_hbm, kt, vt, wq, wo, wr_hbm, wg, wu, wd, gw_hbm, out_ref,
            x_v, wr_v, gw_v, ring, wq_v, wo_v, wg_v, wu_v, wd_v, q_v, o_v, s_v, acc_v,
            ring_sem, small_sem, wq_sem, wo_sem, ffn_sem):

  def kv_block(src, j, half, slot):
    descs = []
    for a in range(0, PD, 8):
      sr = j * PD + a
      if not isinstance(sr, int):
        sr = pl.multiple_of(sr, 8)
      descs.append(_piece(src, ring.at[slot], ring_sem.at[slot], sr, SK - W + HW * half, a, 0, 8, HW))
    return _Group(descs, [(ring.at[slot], ring_sem.at[slot])])

  small = [pltpu.make_async_copy(s, d, small_sem.at[i])
           for i, (s, d) in enumerate([(x_hbm, x_v), (wr_hbm, wr_v), (gw_hbm, gw_v)])]
  g_g = _rows_group(wg, wg_v, ffn_sem.at[0], 0, D // 8, 8, F, GU_S)
  g_u = _rows_group(wu, wu_v, ffn_sem.at[1], 0, D // 8, 8, F, GU_S)
  g_gu = _Group([d for two in zip(g_g.descs, g_u.descs) for d in two], g_g.waits + g_u.waits)
  g_d = _rows_group(wd, wd_v, ffn_sem.at[2], 0, F // WR, WR, D, WD_S)
  g_q = [_rows_group(wq, wq_v, wq_sem.at[g], g * (D // WQ_NG), 240 // WQ_NG, 8, 2048, WQ_S)
         for g in range(WQ_NG)]
  fill = [kv_block(kt, 0, 0, 0), kv_block(kt, 0, 1, 1), kv_block(vt, 0, 0, 2), kv_block(vt, 0, 1, 3)]
  g_o = []
  r0 = 0
  for gi, (n, stride) in enumerate(WO_GROUPS):
    g_o.append((_rows_group(wo, wo_v, wo_sem.at[gi], r0, n, WR, D, stride), r0, WR * n))
    r0 += WR * n

  stream = [g_gu, g_d] + g_q + fill
  state = dict(next=0, inflight=0)

  def pump(once=False):
    while state['next'] < len(stream) and state['inflight'] + stream[state['next']].n <= CAP:
      grp = stream[state['next']]
      grp.issue()
      state['inflight'] += grp.n
      state['next'] += 1
      if once:
        break

  def consume(grp):
    grp.wait()
    state['inflight'] -= grp.n
    pump()

  pump(once=True)
  for c in small:
    c.start()
  pump()
  for c in small:
    c.wait()
  x1 = x_v[...]
  x8 = jnp.broadcast_to(x1.astype(F32), (M, D)).astype(BF)

  consume(g_gu)
  hg = _rnd(jnp.dot(x8, wg_v[...], preferred_element_type=F32))
  hu = _rnd(jnp.dot(x8, wu_v[...], preferred_element_type=F32))
  gub = (_rnd(hg * _rnd(jax.nn.sigmoid(hg))) * hu).astype(BF)
  consume(g_d)
  y = _rnd(jnp.dot(gub, wd_v[...], preferred_element_type=F32))

  for grp in g_q:
    consume(grp)
  q_v[...] = jnp.dot(x8, wq_v[...], preferred_element_type=F32)
  assert state['next'] == len(stream)

  row = lax.broadcasted_iota(jnp.int32, (M, PD), 0)
  col = lax.broadcasted_iota(jnp.int32, (M, PD), 1)
  own = (row < M // 2) == (col < DH)
  wo_descs = [d for (grp, _, _) in g_o for d in grp.descs]
  per = len(wo_descs) // NS

  def refill(j, src, half, slot):
    @pl.when(j + 1 < NP)
    def _():
      kv_block(src, j + 1, half, slot).issue()

    @pl.when(j + 1 == NP)
    def _():
      _start_all(wo_descs[slot * per:(slot + 1) * per], slot * per)

  def pair(j, carry):
    c0 = pl.multiple_of(j * PD, 128)
    qm = jnp.where(own, q_v[:, pl.ds(c0, PD)], 0.0).astype(BF)
    for half in range(2):
      slot = half
      _wait_all(ring.at[slot], ring_sem.at[slot])
      s_v[:, HW * half:HW * (half + 1)] = jnp.dot(qm, ring[slot], preferred_element_type=F32)
      refill(j, kt, half, slot)
    s = _rnd(_rnd(s_v[...]) * SCALE)
    m = jnp.max(s, axis=1, keepdims=True)
    eb = jnp.exp(s - m).astype(BF)
    inv = 1.0 / jnp.sum(eb.astype(F32), axis=1, keepdims=True)
    for half in range(2):
      slot = 2 + half
      _wait_all(ring.at[slot], ring_sem.at[slot])
      d = lax.dot_general(eb[:, HW * half:HW * (half + 1)], ring[slot], NT, preferred_element_type=F32)
      if half == 0:
        o_v[:, pl.ds(c0, PD)] = d
      else:
        o_v[:, pl.ds(c0, PD)] = jnp.where(own, (o_v[:, pl.ds(c0, PD)] + d) * inv, 0.0)
      refill(j, vt, half, slot)
    return carry

  lax.fori_loop(0, NP, pair, 0)

  xf = x1.astype(F32)
  wr = wr_v[...].astype(F32)
  gw = gw_v[...].astype(F32)
  racc = jnp.zeros((1, 128), F32)
  gacc = jnp.zeros((1, 128), F32)
  for i in range(D // 128):
    xi = xf[:, 128 * i:128 * (i + 1)]
    racc = racc + xi * wr[i:i + 1, :]
    gacc = gacc + _rnd(xi * gw[i:i + 1, :])
  r_sel = _rnd(jax.nn.sigmoid(_rnd(jnp.sum(racc, axis=1, keepdims=True))))
  g = _rnd(jax.nn.sigmoid(_rnd(jnp.sum(gacc, axis=1, keepdims=True))))
  upd = _rnd(xf * 0.0 + _rnd(y[0:1] * r_sel))
  t2 = _rnd(_rnd(1.0 - g) * _rnd(xf + upd))

  for gi, (grp, r0, nr) in enumerate(g_o):
    grp.wait()
    d = jnp.dot(o_v[:, r0:r0 + nr].astype(BF), wo_v[pl.ds(r0, nr), :], preferred_element_type=F32)
    if gi == 0:
      acc_v[...] = d
    elif gi < len(g_o) - 1:
      acc_v[...] += d
    else:
      acc = acc_v[...] + d
  a = _rnd(acc[0:1] + acc[M // 2:M // 2 + 1])
  out_ref[...] = (_rnd(g * a) + t2).astype(BF)


@jax.jit
def pallas_gated_mix__sliding_block_cached__moe_arch_mod__decode_kernel(
    A_x: jax.Array,
    A_k_cache: jax.Array,
    A_v_cache: jax.Array,
    A_wq: jax.Array,
    A_wo: jax.Array,
    B_x: jax.Array,
    B_w_r: jax.Array,
    B_w_gate: jax.Array,
    B_w_up: jax.Array,
    B_w_down: jax.Array,
    gate_w: jax.Array,
):
  del B_x
  kt = jnp.swapaxes(A_k_cache[0], 1, 2).reshape(H * DH, SK)
  vt = jnp.swapaxes(A_v_cache[0], 1, 2).reshape(H * DH, SK)
  hbm = pl.BlockSpec(memory_space=pltpu.HBM)
  out = pl.pallas_call(
      _kernel,
      out_shape=jax.ShapeDtypeStruct((1, D), BF),
      in_specs=[hbm] * 10,
      out_specs=pl.BlockSpec(memory_space=pltpu.VMEM),
      scratch_shapes=[
          pltpu.VMEM((1, D), BF), pltpu.VMEM((5, 128), BF), pltpu.VMEM((5, 128), BF),
          pltpu.VMEM((NS, PD, HW), BF),
          pltpu.VMEM((D, H * DH), BF), pltpu.VMEM((H * DH, D), BF),
          pltpu.VMEM((D, F), BF), pltpu.VMEM((D, F), BF), pltpu.VMEM((F, D), BF),
          pltpu.VMEM((M, H * DH), F32), pltpu.VMEM((M, H * DH), F32),
          pltpu.VMEM((M, W), F32), pltpu.VMEM((M, D), F32),
          pltpu.SemaphoreType.DMA((NS,)), pltpu.SemaphoreType.DMA((3,)),
          pltpu.SemaphoreType.DMA((WQ_NG,)), pltpu.SemaphoreType.DMA((len(WO_GROUPS),)),
          pltpu.SemaphoreType.DMA((3,)),
      ],
      compiler_params=pltpu.CompilerParams(
          vmem_limit_bytes=64 * 1024 * 1024, disable_semaphore_checks=True),
      name="gated_mix_decode",
  )(A_x.reshape(1, D), kt, vt, A_wq, A_wo, B_w_r.reshape(5, 128), B_w_gate, B_w_up, B_w_down,
    gate_w.reshape(5, 128))
  return out.reshape(1, 1, D)
```
